```python
import os as _os
_os.environ.setdefault("JAX_PLATFORMS", "cpu")
import jax
import jax.numpy as jnp

def _softmax(x, axis=-1):
    return jax.nn.softmax(x, axis=axis)
def _gelu(x):
    return jax.nn.gelu(x, approximate=True)
def _silu(x):
    return jax.nn.silu(x)
def _sigmoid(x):
    return jax.nn.sigmoid(x)
def _layernorm(x, axis=-1, eps=1e-5):
    m = jnp.mean(x, axis=axis, keepdims=True)
    v = jnp.var(x, axis=axis, keepdims=True)
    return (x - m) / jnp.sqrt(v + eps)
def _scatter_add(tgt, idx, src, axis=0):
    return tgt.at[idx].add(src)
def _segment_sum(src, seg, n):
    return jax.ops.segment_sum(src, seg, n)
class _Rng:
    def __init__(self, key):
        self._k = key
    def _next(self):
        self._k, sub = jax.random.split(self._k)
        return sub
    def normal(self, shape):
        return jax.random.normal(self._next(), shape, dtype=jnp.bfloat16)
    def randint(self, lo, hi, shape):
        return jax.random.randint(self._next(), shape, lo, hi, dtype=jnp.int32)
    def uniform(self, shape, lo=0.0, hi=1.0):
        return jax.random.uniform(self._next(), shape, jnp.bfloat16, lo, hi)
    def permutation(self, n):
        return jax.random.permutation(self._next(), n)


kernel_name = 'gated_mix__gqa_block_cached__dense_activation_squared_relu__decode'

def setup_inputs():
    _rng = _Rng(jax.random.key(int.from_bytes(__import__("os").urandom(4), "little")))
    _w = (lambda a: (lambda t: t.astype(jnp.bfloat16) if jnp.issubdtype(t.dtype, jnp.floating) else t)(jnp.asarray(a)))
    def _A_setup():
        B, Sq, D = 4, 1, 512
        Hq, Hkv, Sk, Dh = 32, 8, 4096, 128
        assert Hq % Hkv == 0, (Hq, Hkv)
        return {
            "x": _w((lambda *s: _rng.normal(s) * 0.05)(B, Sq, D)),
            "k_cache": _w((lambda *s: _rng.normal(s) * 3.2)(B, Hkv, Sk, Dh)),
            "v_cache": _w((lambda *s: _rng.normal(s) * 1.6)(B, Hkv, Sk, Dh)),
            "wq": _w((lambda *s: _rng.normal(s) * 3.2)(D, Hq * Dh) * (D ** -0.5)),
            "wo": _w((lambda *s: _rng.normal(s) * 1.6)(Hq * Dh, D) * ((Hq * Dh) ** -0.5)),
        }
    _A_in = _A_setup()

    def _B_setup():
        B, S, D, F = 4, 1, 512, 1792
        return {
            "x": _w((lambda *s: _rng.normal(s) * 0.05)(B, S, D)),
            "w1": _w((lambda *s: _rng.normal(s) * 0.1)(D, F)),
            "b1": _w((lambda *s: _rng.normal(s) * 0.05)(F)),
            "w2": _w((lambda *s: _rng.normal(s) * 0.05)(F, D)),
            "b2": _w((lambda *s: _rng.normal(s) * 0.05)(D)),
        }
    _B_in = _B_setup()

    return {
        "A_x": _A_in["x"],
        "A_k_cache": _A_in["k_cache"],
        "A_v_cache": _A_in["v_cache"],
        "A_wq": _A_in["wq"],
        "A_wo": _A_in["wo"],
        "B_x": _B_in["x"],
        "B_w1": _B_in["w1"],
        "B_b1": _B_in["b1"],
        "B_w2": _B_in["w2"],
        "B_b2": _B_in["b2"],
        "gate_w": _w((lambda *s: _rng.normal(s) * 0.05)(512) * 16.0),
    }

def reference(A_x, A_k_cache, A_v_cache, A_wq, A_wo, B_x, B_w1, B_b1, B_w2, B_b2, gate_w):
    def _A_ref(x, k_cache, v_cache, wq, wo):
        B, Sq, D = x.shape
        Hq, Dh = 32, 128
        Hkv = k_cache.shape[1]
        rep = Hq // Hkv
        q = (lambda x, *d: x.transpose(*d))((x @ wq).reshape(B, Sq, Hq, Dh), 0, 2, 1, 3)
        k = jnp.repeat(k_cache, rep, axis=1)
        v = jnp.repeat(v_cache, rep, axis=1)
        scores = jnp.einsum("bhqd,bhkd->bhqk", q, k) * (Dh ** -0.5)
        p = _softmax(scores, axis=-1)
        o = jnp.einsum("bhqk,bhkd->bhqd", p, v)
        return (lambda x, *d: x.transpose(*d))(o, 0, 2, 1, 3).reshape(B, Sq, Hq * Dh) @ wo

    def _B_ref(x, w1, b1, w2, b2):
        h = jnp.einsum("bsd,df->bsf", x, w1) + b1
        zero = jnp.zeros_like(h)
        r = jnp.where(h > zero, h, zero)
        h = r * r
        out = jnp.einsum("bsf,fd->bsd", h, w2) + b2
        return out

    x = A_x
    g = _sigmoid((x * gate_w).sum(-1, keepdims=True))
    a = _A_ref(x, A_k_cache, A_v_cache, A_wq, A_wo)
    b = _B_ref(x, B_w1, B_b1, B_w2, B_b2)
    return g * a + (1 - g) * b
```

```python
import jax
import jax.numpy as jnp
from jax import lax
import jax.experimental.pallas as pl
import jax.experimental.pallas.tpu as pltpu

_F32 = jnp.float32
_BF16 = jnp.bfloat16


@jax.jit
def pallas_gated_mix__gqa_block_cached__dense_activation_squared_relu__decode_kernel(
    A_x: jax.Array,
    A_k_cache: jax.Array,
    A_v_cache: jax.Array,
    A_wq: jax.Array,
    A_wo: jax.Array,
    B_x: jax.Array,
    B_w1: jax.Array,
    B_b1: jax.Array,
    B_w2: jax.Array,
    B_b2: jax.Array,
    gate_w: jax.Array,
):
    B, Sq, D = A_x.shape
    _, Hkv, Sk, Dh = A_k_cache.shape
    HD = A_wq.shape[1]
    Hq = HD // Dh
    rep = Hq // Hkv
    F = B_w1.shape[1]
    assert Sq == 1 and rep <= 8
    n_steps = B * Hkv
    scale = float(Dh) ** -0.5

    x2 = A_x.reshape(B, D)
    k3 = A_k_cache.reshape(B * Hkv, Sk, Dh)
    v3 = A_v_cache.reshape(B * Hkv, Sk, Dh)
    b1_2 = B_b1.reshape(1, F)
    b2_2 = B_b2.reshape(1, D)
    gw_2 = gate_w.reshape(1, D)

    def kernel(x_ref, k_ref, v_ref, wq_ref, wo_ref, w1_ref, b1_ref, w2_ref,
               b2_ref, gw_ref, out_ref, q_scr, o_scr, oall_scr, ffn_scr, g_scr):
        step = pl.program_id(0)

        @pl.when(step == 0)
        def _prologue():
            x = x_ref[...]
            q = jnp.dot(x, wq_ref[...], preferred_element_type=_F32)
            q = q.astype(_BF16).astype(_F32)
            q_scr[...] = jnp.zeros(q_scr.shape, _F32)
            for b in range(B):
                for hq in range(Hq):
                    h, r = divmod(hq, rep)
                    row = (b * Hkv + h) * 8 + r
                    q_scr[row:row + 1, :] = q[b:b + 1, hq * Dh:(hq + 1) * Dh]
            hid = jnp.dot(x, w1_ref[...], preferred_element_type=_F32)
            hid = hid + b1_ref[...].astype(_F32)
            hid = jnp.maximum(hid, 0.0)
            hid = hid * hid
            ffn = jnp.dot(hid.astype(_BF16), w2_ref[...],
                          preferred_element_type=_F32)
            ffn_scr[...] = ffn + b2_ref[...].astype(_F32)
            gl = jnp.sum(x.astype(_F32) * gw_ref[...].astype(_F32), axis=-1,
                         keepdims=True)
            g_scr[...] = 1.0 / (1.0 + jnp.exp(-gl))

        q8 = q_scr[pl.ds(pl.multiple_of(step * 8, 8), 8), :].astype(_BF16)
        k = k_ref[...]
        s = lax.dot_general(q8, k, (((1,), (1,)), ((), ())),
                            preferred_element_type=_F32) * scale
        m = jnp.max(s, axis=-1, keepdims=True)
        p = jnp.exp(s - m)
        l = jnp.sum(p, axis=-1, keepdims=True)
        o = jnp.dot(p.astype(_BF16), v_ref[...], preferred_element_type=_F32)
        o_scr[pl.ds(pl.multiple_of(step * 8, 8), 8), :] = o / l

        @pl.when(step == n_steps - 1)
        def _epilogue():
            for b in range(B):
                for hq in range(Hq):
                    h, r = divmod(hq, rep)
                    row = (b * Hkv + h) * 8 + r
                    oall_scr[b:b + 1, hq * Dh:(hq + 1) * Dh] = o_scr[row:row + 1, :]
            oall = oall_scr[...].astype(_BF16)
            a = jnp.dot(oall, wo_ref[...], preferred_element_type=_F32)
            g = g_scr[...]
            out_ref[...] = (g * a + (1.0 - g) * ffn_scr[...]).astype(out_ref.dtype)

    const = lambda i: (0, 0)
    out = pl.pallas_call(
        kernel,
        grid=(n_steps,),
        in_specs=[
            pl.BlockSpec((B, D), const),
            pl.BlockSpec((None, Sk, Dh), lambda i: (i, 0, 0)),
            pl.BlockSpec((None, Sk, Dh), lambda i: (i, 0, 0)),
            pl.BlockSpec((D, HD), const),
            pl.BlockSpec((HD, D), const),
            pl.BlockSpec((D, F), const),
            pl.BlockSpec((1, F), const),
            pl.BlockSpec((F, D), const),
            pl.BlockSpec((1, D), const),
            pl.BlockSpec((1, D), const),
        ],
        out_specs=pl.BlockSpec((B, D), const),
        out_shape=jax.ShapeDtypeStruct((B, D), A_x.dtype),
        scratch_shapes=[
            pltpu.VMEM((n_steps * 8, Dh), _F32),
            pltpu.VMEM((n_steps * 8, Dh), _F32),
            pltpu.VMEM((B, HD), _F32),
            pltpu.VMEM((B, D), _F32),
            pltpu.VMEM((B, 1), _F32),
        ],
        compiler_params=pltpu.CompilerParams(
            dimension_semantics=("arbitrary",),
            vmem_limit_bytes=96 * 1024 * 1024,
        ),
    )(x2, k3, v3, A_wq, A_wo, B_w1, b1_2, B_w2, b2_2, gw_2)
    return out.reshape(B, Sq, D)
```

```python
import jax
import jax.numpy as jnp
from jax import lax
import jax.experimental.pallas as pl
import jax.experimental.pallas.tpu as pltpu

_F32 = jnp.float32
_BF16 = jnp.bfloat16
_RING = 3


@jax.jit
def pallas_gated_mix__gqa_block_cached__dense_activation_squared_relu__decode_kernel(
    A_x: jax.Array,
    A_k_cache: jax.Array,
    A_v_cache: jax.Array,
    A_wq: jax.Array,
    A_wo: jax.Array,
    B_x: jax.Array,
    B_w1: jax.Array,
    B_b1: jax.Array,
    B_w2: jax.Array,
    B_b2: jax.Array,
    gate_w: jax.Array,
):
    B, Sq, D = A_x.shape
    _, Hkv, Sk, Dh = A_k_cache.shape
    HD = A_wq.shape[1]
    Hq = HD // Dh
    rep = Hq // Hkv
    F = B_w1.shape[1]
    G = rep * Dh
    n_steps = B * Hkv
    R = _RING
    assert Sq == 1 and rep <= 8 and n_steps > R and B >= 2
    scale = float(Dh) ** -0.5

    x2 = A_x.reshape(B, D)
    k3 = A_k_cache.reshape(B * Hkv, Sk, Dh)
    v3 = A_v_cache.reshape(B * Hkv, Sk, Dh)

    def kernel(x_hbm, b1_hbm, b2_hbm, gw_hbm, k_hbm, v_hbm, wq_hbm, wo_hbm,
               w1_hbm, w2_hbm,
               out_ref,
               x_ref, b1_ref, b2_ref, gw_ref,
               kbuf, vbuf, wq_buf, wo_buf, w1_buf, w2_buf,
               q_scr, oall_scr, acc_scr, g_scr,
               ssem, ksem, vsem, wsem):
        step = pl.program_id(0)
        h = step // B
        b = step % B
        slot = step % R

        def kv_index(s):
            return (s % B) * Hkv + s // B

        def kcopy(s, sl):
            return pltpu.make_async_copy(k_hbm.at[kv_index(s)], kbuf.at[sl],
                                         ksem.at[sl])

        def vcopy(s, sl):
            return pltpu.make_async_copy(v_hbm.at[kv_index(s)], vbuf.at[sl],
                                         vsem.at[sl])

        wq_cp = pltpu.make_async_copy(wq_hbm, wq_buf, wsem.at[0])
        wo_cp = pltpu.make_async_copy(wo_hbm, wo_buf, wsem.at[1])
        w1_cp = pltpu.make_async_copy(w1_hbm, w1_buf, wsem.at[2])
        w2_cp = pltpu.make_async_copy(w2_hbm, w2_buf, wsem.at[3])

        @pl.when(step == 0)
        def _prologue():
            wq_cp.start()
            for s in range(R):
                kcopy(s, s).start()
                vcopy(s, s).start()
            small = [
                pltpu.make_async_copy(src, dst, ssem.at[i])
                for i, (src, dst) in enumerate(
                    [(x_hbm, x_ref), (b1_hbm, b1_ref), (b2_hbm, b2_ref),
                     (gw_hbm, gw_ref)])
            ]
            for c in small:
                c.start()
            w1_cp.start()
            w2_cp.start()
            for c in small:
                c.wait()
            wq_cp.wait()
            wo_cp.start()
            x = x_ref[...]
            q = jnp.dot(x, wq_buf[...], preferred_element_type=_F32)
            q = q.astype(_BF16).astype(_F32)
            q_scr[...] = jnp.zeros(q_scr.shape, _F32)
            for bb in range(B):
                for hq in range(Hq):
                    hh, r = divmod(hq, rep)
                    row = (hh * B + bb) * 8 + r
                    q_scr[row:row + 1, :] = q[bb:bb + 1, hq * Dh:(hq + 1) * Dh]
            gl = jnp.sum(x.astype(_F32) * gw_ref[...].astype(_F32)[None, :],
                         axis=-1, keepdims=True)
            g_scr[...] = 1.0 / (1.0 + jnp.exp(-gl))

        q8 = q_scr[pl.ds(pl.multiple_of(step * 8, 8), 8), :].astype(_BF16)
        kcopy(step, slot).wait()
        s = lax.dot_general(q8, kbuf[slot], (((1,), (1,)), ((), ())),
                            preferred_element_type=_F32) * scale

        @pl.when(step + R < n_steps)
        def _():
            kcopy(step + R, slot).start()

        m = jnp.max(s, axis=-1, keepdims=True)
        p = jnp.exp(s - m)
        l = jnp.sum(p, axis=-1, keepdims=True)
        vcopy(step, slot).wait()
        o = jnp.dot(p.astype(_BF16), vbuf[slot],
                    preferred_element_type=_F32) / l

        @pl.when(step + R < n_steps)
        def _():
            vcopy(step + R, slot).start()

        for bb in range(B):
            @pl.when(b == bb)
            def _():
                for r in range(rep):
                    oall_scr[bb:bb + 1, r * Dh:(r + 1) * Dh] = o[r:r + 1, :]

        @pl.when(step == 1)
        def _ffn():
            w1_cp.wait()
            w2_cp.wait()
            x = x_ref[...]
            hid = jnp.dot(x, w1_buf[...], preferred_element_type=_F32)
            hid = hid + b1_ref[...].astype(_F32)[None, :]
            hid = jnp.maximum(hid, 0.0)
            hid = hid * hid
            ffn = jnp.dot(hid.astype(_BF16), w2_buf[...],
                          preferred_element_type=_F32)
            ffn = ffn + b2_ref[...].astype(_F32)[None, :]
            acc_scr[...] = (1.0 - g_scr[...]) * ffn

        @pl.when(step == B - 1)
        def _():
            wo_cp.wait()

        @pl.when(b == B - 1)
        def _proj():
            wo_blk = wo_buf[pl.ds(pl.multiple_of(h * G, G), G), :]
            a = jnp.dot(oall_scr[...].astype(_BF16), wo_blk,
                        preferred_element_type=_F32)
            acc_scr[...] += g_scr[...] * a

        @pl.when(step == n_steps - 1)
        def _():
            out_ref[...] = acc_scr[...].astype(out_ref.dtype)

    anyspec = pl.BlockSpec(memory_space=pl.ANY)
    out = pl.pallas_call(
        kernel,
        grid=(n_steps,),
        in_specs=[anyspec] * 10,
        out_specs=pl.BlockSpec((B, D), lambda i: (0, 0)),
        out_shape=jax.ShapeDtypeStruct((B, D), A_x.dtype),
        scratch_shapes=[
            pltpu.VMEM((B, D), _BF16),
            pltpu.VMEM((F,), _BF16),
            pltpu.VMEM((D,), _BF16),
            pltpu.VMEM((D,), _BF16),
            pltpu.VMEM((R, Sk, Dh), _BF16),
            pltpu.VMEM((R, Sk, Dh), _BF16),
            pltpu.VMEM((D, HD), _BF16),
            pltpu.VMEM((HD, D), _BF16),
            pltpu.VMEM((D, F), _BF16),
            pltpu.VMEM((F, D), _BF16),
            pltpu.VMEM((n_steps * 8, Dh), _F32),
            pltpu.VMEM((B, G), _F32),
            pltpu.VMEM((B, D), _F32),
            pltpu.VMEM((B, 1), _F32),
            pltpu.SemaphoreType.DMA((4,)),
            pltpu.SemaphoreType.DMA((R,)),
            pltpu.SemaphoreType.DMA((R,)),
            pltpu.SemaphoreType.DMA((4,)),
        ],
        compiler_params=pltpu.CompilerParams(
            dimension_semantics=("arbitrary",),
            vmem_limit_bytes=96 * 1024 * 1024,
        ),
    )(x2, B_b1, B_b2, gate_w, k3, v3, A_wq, A_wo, B_w1, B_w2)
    return out.reshape(B, Sq, D)
```
